```python
import os as _os
_os.environ.setdefault("JAX_PLATFORMS", "cpu")
import jax
import jax.numpy as jnp

def _softmax(x, axis=-1):
    return jax.nn.softmax(x, axis=axis)
def _gelu(x):
    return jax.nn.gelu(x, approximate=True)
def _silu(x):
    return jax.nn.silu(x)
def _sigmoid(x):
    return jax.nn.sigmoid(x)
def _layernorm(x, axis=-1, eps=1e-5):
    m = jnp.mean(x, axis=axis, keepdims=True)
    v = jnp.var(x, axis=axis, keepdims=True)
    return (x - m) / jnp.sqrt(v + eps)
def _scatter_add(tgt, idx, src, axis=0):
    return tgt.at[idx].add(src)
def _segment_sum(src, seg, n):
    return jax.ops.segment_sum(src, seg, n)
class _Rng:
    def __init__(self, key):
        self._k = key
    def _next(self):
        self._k, sub = jax.random.split(self._k)
        return sub
    def normal(self, shape):
        return jax.random.normal(self._next(), shape, dtype=jnp.bfloat16)
    def randint(self, lo, hi, shape):
        return jax.random.randint(self._next(), shape, lo, hi, dtype=jnp.int32)
    def uniform(self, shape, lo=0.0, hi=1.0):
        return jax.random.uniform(self._next(), shape, jnp.bfloat16, lo, hi)
    def permutation(self, n):
        return jax.random.permutation(self._next(), n)


kernel_name = 'standalone__gqa_block_cached__near_ridge'

def setup_inputs():
    _rng = _Rng(jax.random.key(int.from_bytes(__import__("os").urandom(4), "little")))
    _w = (lambda a: (lambda t: t.astype(jnp.bfloat16) if jnp.issubdtype(t.dtype, jnp.floating) else t)(jnp.asarray(a)))
    B, Sq, D = 8, 64, 512
    Hq, Hkv, Sk, Dh = 32, 8, 64, 128
    assert Hq % Hkv == 0, (Hq, Hkv)
    return {
        "x": _w((lambda *s: _rng.normal(s) * 0.8)(B, Sq, D)),
        "k_cache": _w((lambda *s: _rng.normal(s) * 0.8)(B, Hkv, Sk, Dh)),
        "v_cache": _w((lambda *s: _rng.normal(s) * 0.05)(B, Hkv, Sk, Dh)),
        "wq": _w((lambda *s: _rng.normal(s) * 0.8)(D, Hq * Dh) * (D ** -0.5)),
        "wo": _w((lambda *s: _rng.normal(s) * 0.05)(Hq * Dh, D) * ((Hq * Dh) ** -0.5)),
    }

def reference(x, k_cache, v_cache, wq, wo):
    B, Sq, D = x.shape
    Hq, Dh = 32, 128
    Hkv = k_cache.shape[1]
    rep = Hq // Hkv
    q = (lambda x, *d: x.transpose(*d))((x @ wq).reshape(B, Sq, Hq, Dh), 0, 2, 1, 3)
    k = jnp.repeat(k_cache, rep, axis=1)
    v = jnp.repeat(v_cache, rep, axis=1)
    scores = jnp.einsum("bhqd,bhkd->bhqk", q, k) * (Dh ** -0.5)
    p = _softmax(scores, axis=-1)
    o = jnp.einsum("bhqk,bhkd->bhqd", p, v)
    return (lambda x, *d: x.transpose(*d))(o, 0, 2, 1, 3).reshape(B, Sq, Hq * Dh) @ wo
```

```python
import functools
import math
import jax
import jax.numpy as jnp
import jax.experimental.pallas as pl
import jax.experimental.pallas.tpu as pltpu


@jax.jit
def pallas_standalone__gqa_block_cached__near_ridge_kernel(x, k_cache, v_cache, wq, wo):
    B, Sq, D = x.shape
    _, Hkv, Sk, Dh = k_cache.shape
    Hq = wq.shape[1] // Dh
    rep = Hq // Hkv
    T = B * Sq
    G = rep * Dh
    NC = 128
    NCH = G // NC
    exp2_scale = (Dh ** -0.5) * math.log2(math.e)

    barriers = {0: (0,), 1: (1,), 2: (2,), 3: (3, 4), 5: (5, 6, 7), 7: (8, 9)}
    sem_of = {}
    for i, (stage, bs) in enumerate(sorted(barriers.items())):
        for s in bs:
            sem_of[s] = i
    n_sems = len(barriers) + 1
    starts = {(1, 5): 3, (2, 3): 4, (2, 7): 5, (3, 4): 6, (4, 0): 7, (4, 4): 8, (4, 7): 9}

    def kernel_function(x_hbm, k_hbm, v_hbm, wq_hbm, wo_hbm, out_hbm,
                        x_v, k_v, v_v, wq_v, wo_v, q_a, q_b, o_a, o_b, acc, out_v, sems):
        def batch(s):
            sem = sems.at[sem_of[s]]
            cps = []
            if s == 0:
                cps.append(pltpu.make_async_copy(x_hbm, x_v, sem))
            if s < Hkv:
                cps.append(pltpu.make_async_copy(
                    wq_hbm.at[:, pl.ds(s * G, G)], wq_v.at[s], sem))
            if 1 <= s <= Hkv:
                cps.append(pltpu.make_async_copy(k_hbm.at[:, s - 1], k_v.at[s - 1], sem))
                cps.append(pltpu.make_async_copy(v_hbm.at[:, s - 1], v_v.at[s - 1], sem))
            if s >= 2:
                cps.append(pltpu.make_async_copy(
                    wo_hbm.at[pl.ds((s - 2) * G, G), :], wo_v.at[s - 2], sem))
            return cps

        def cp_out(c):
            sl = pl.ds(c * NC, NC)
            return pltpu.make_async_copy(out_v.at[:, sl], out_hbm.at[:, sl], sems.at[n_sems - 1])

        def start(s):
            for c in batch(s):
                c.start()

        def wait(*ss):
            for s in ss:
                for c in batch(s):
                    c.wait()

        q_bufs = (q_a, q_b)
        o_bufs = (o_a, o_b)

        def B_chunk(g, c, r0=0, r1=T):
            sl = slice(c * NC, (c + 1) * NC)
            q = jnp.dot(x_v[r0:r1, :], wq_v[g, :, sl], preferred_element_type=jnp.float32)
            q_bufs[g % 2][r0:r1, sl] = q.astype(jnp.bfloat16)

        def A_S(g, b):
            q_ref = q_bufs[g % 2]
            Q = jnp.concatenate(
                [q_ref[b * Sq:(b + 1) * Sq, j * Dh:(j + 1) * Dh] for j in range(rep)], axis=0)
            k = k_v[g, b]
            st = jax.lax.dot_general(k, Q, (((1,), (1,)), ((), ())),
                                     preferred_element_type=jnp.float32)
            m = jnp.max(st, axis=0, keepdims=True)
            e = jnp.exp2((st - m) * exp2_scale)
            l = jnp.sum(e, axis=0, keepdims=True)
            return (e * (1.0 / l)).astype(jnp.bfloat16).T

        def A_PV(g, b, p):
            o_ref = o_bufs[g % 2]
            v = v_v[g, b]
            for j in range(rep):
                O = jnp.dot(p[j * Sq:(j + 1) * Sq, :], v, preferred_element_type=jnp.float32)
                o_ref[b * Sq:(b + 1) * Sq, j * Dh:(j + 1) * Dh] = O.astype(jnp.bfloat16)

        def C_chunk(g, c, r0=0, r1=T):
            sl = slice(c * NC, (c + 1) * NC)
            contrib = jnp.dot(o_bufs[g % 2][r0:r1, :], wo_v[g, :, sl], preferred_element_type=jnp.float32)
            if g == 0:
                acc[r0:r1, sl] = contrib
            elif g < Hkv - 1:
                acc[r0:r1, sl] += contrib
            else:
                out_v[r0:r1, sl] = (acc[r0:r1, sl] + contrib).astype(out_v.dtype)

        def fillers(s):
            fs = []
            if s == 1 or s == Hkv:
                fn, g = (B_chunk, s) if s == 1 else (C_chunk, s - 2)
                for h in range(2):
                    for c in range(NCH):
                        fs.append(functools.partial(fn, g, c, h * (T // 2), (h + 1) * (T // 2)))
            else:
                if s < Hkv:
                    for c in range(NCH):
                        fs.append(functools.partial(B_chunk, s, c))
                if s >= 2:
                    for c in range(NCH):
                        fs.append(functools.partial(C_chunk, s - 2, c))
            return fs

        start(0)
        wait(*barriers[0])
        start(1)
        for c in range(NCH):
            if c == NCH - 1:
                start(2)
            B_chunk(0, c)

        p_vals = {}
        for s in range(1, Hkv + 2):
            if s in barriers:
                wait(*barriers[s])
            fs = fillers(s)
            if s <= Hkv:
                a = s - 1
                for b in range(2):
                    if (a, b) not in p_vals:
                        p_vals[(a, b)] = A_S(a, b)
                for i in range(B):
                    if (s, i) in starts:
                        start(starts[(s, i)])
                    nb = i + 2
                    if nb < B:
                        p_vals[(a, nb)] = A_S(a, nb)
                    elif a + 1 < Hkv and (s + 1) not in barriers:
                        p_vals[(a + 1, nb - B)] = A_S(a + 1, nb - B)
                    fs[i]()
                    A_PV(a, i, p_vals.pop((a, i)))
            else:
                for c, f in enumerate(fs):
                    f()
                    cp_out(c).start()
        for c in range(NCH):
            cp_out(c).wait()

    x2 = x.reshape(T, D)
    bf = jnp.bfloat16
    out = pl.pallas_call(
        kernel_function,
        in_specs=[pl.BlockSpec(memory_space=pl.ANY)] * 5,
        out_specs=pl.BlockSpec(memory_space=pl.ANY),
        out_shape=jax.ShapeDtypeStruct((T, D), x.dtype),
        scratch_shapes=[
            pltpu.VMEM((T, D), bf),
            pltpu.VMEM((Hkv, B, Sk, Dh), bf),
            pltpu.VMEM((Hkv, B, Sk, Dh), bf),
            pltpu.VMEM((Hkv, D, G), bf),
            pltpu.VMEM((Hkv, G, D), bf),
            pltpu.VMEM((T, G), bf),
            pltpu.VMEM((T, G), bf),
            pltpu.VMEM((T, G), bf),
            pltpu.VMEM((T, G), bf),
            pltpu.VMEM((T, D), jnp.float32),
            pltpu.VMEM((T, D), bf),
            pltpu.SemaphoreType.DMA((n_sems,)),
        ],
        compiler_params=pltpu.CompilerParams(
            vmem_limit_bytes=96 * 1024 * 1024,
        ),
    )(x2, k_cache, v_cache, wq, wo)
    return out.reshape(B, Sq, D)
```

```python
import functools
import math
import jax
import jax.numpy as jnp
import jax.experimental.pallas as pl
import jax.experimental.pallas.tpu as pltpu


@jax.jit
def pallas_standalone__gqa_block_cached__near_ridge_kernel(x, k_cache, v_cache, wq, wo):
    B, Sq, D = x.shape
    _, Hkv, Sk, Dh = k_cache.shape
    Hq = wq.shape[1] // Dh
    rep = Hq // Hkv
    T = B * Sq
    G = rep * Dh
    NC = 128 if (G % 128 == 0 and D % 128 == 0) else min(G, D)
    NCQ = G // NC
    NCO = D // NC
    assert G % NC == 0 and D % NC == 0 and D % 2 == 0 and Hkv >= 2
    KH = D // 2
    RT = T - 128 if T > 128 else T
    exp2_scale = (Dh ** -0.5) * math.log2(math.e)

    n_batches = Hkv + 2
    if Hkv == 8 and B == 8:
        groups = {-1: (-1,), 0: (0,), 1: (1,), 2: (2,), 3: (3, 4), 5: (5, 6, 7), 7: (8, 9)}
        starts = {(1, 5): [3], (2, 3): [4], (2, 7): [5], (3, 4): [6], (4, 0): [7], (4, 4): [8], (4, 7): [9]}
    else:
        groups = {-1: (-1,), 0: (0,), 1: (1,), 2: (2,)}
        s, step = 3, 2
        while s < n_batches:
            groups[s] = tuple(range(s, min(s + step, n_batches)))
            s += step
            step += 1
        starts = {}
        for b in range(3, n_batches):
            first = [st for st, bs in groups.items() if b in bs][0]
            prev = max(st for st in groups if st < first)
            pos = groups[first].index(b)
            starts.setdefault((max(prev, 1), min(B - 1, 4 + pos)), []).append(b)
    barrier_stages = set(groups)
    group_of = {b: st for st, bs in groups.items() for b in bs}
    sem_of = {st: i for i, st in enumerate(sorted(groups))}
    n_sems = len(groups) + 1
    LB = 4
    early_k = {g for g in range(2, Hkv) if (g + 1) in barrier_stages}

    def k_batch(g):
        return g if g in early_k else g + 1

    def kernel_function(x_hbm, k_hbm, v_hbm, wq_hbm, wo_hbm, out_hbm,
                        x_v, k_v, v_v, wq_v, wo_v, q_a, q_b, o_a, o_b, acc, out_v, qpart, sems):
        started = set()
        waited = set()
        ready = set()

        def need(*items):
            for it in items:
                assert it in ready, ("read before its DMA was waited for", it)

        def items_of(s):
            its = []
            if s <= 0:
                its += [("x", s), ("wq0", s)]
            elif s < Hkv:
                its.append(("wq", s))
            its += [("k", g) for g in range(Hkv) if k_batch(g) == s]
            if 1 <= s <= Hkv:
                its.append(("v", s - 1))
            if s >= 2:
                its.append(("wo", s - 2))
            return its

        def copies(s):
            sem = sems.at[sem_of[group_of[s]]]
            cps = []
            if s <= 0:
                ks = pl.ds(0 if s < 0 else KH, KH)
                cps.append(pltpu.make_async_copy(x_hbm.at[:, ks], x_v.at[:, ks], sem))
                cps.append(pltpu.make_async_copy(
                    wq_hbm.at[ks, pl.ds(0, G)], wq_v.at[0, ks, :], sem))
            elif s < Hkv:
                cps.append(pltpu.make_async_copy(
                    wq_hbm.at[:, pl.ds(s * G, G)], wq_v.at[s], sem))
            for g in range(Hkv):
                if k_batch(g) == s:
                    cps.append(pltpu.make_async_copy(k_hbm.at[:, g], k_v.at[g], sem))
            if 1 <= s <= Hkv:
                cps.append(pltpu.make_async_copy(v_hbm.at[:, s - 1], v_v.at[s - 1], sem))
            if s >= 2:
                cps.append(pltpu.make_async_copy(
                    wo_hbm.at[pl.ds((s - 2) * G, G), :], wo_v.at[s - 2], sem))
            return cps

        def start(s):
            assert s not in started
            grp = group_of[s]
            assert all(b in waited for b in group_of if group_of[b] != grp
                       and sem_of[group_of[b]] == sem_of[grp] and b in started)
            started.add(s)
            for c in copies(s):
                c.start()

        def wait_group(st):
            bs = groups[st]
            assert all(b in started and b not in waited for b in bs), ("group incomplete", st)
            for b in bs:
                for c in copies(b):
                    c.wait()
            for b in bs:
                waited.add(b)
                ready.update(items_of(b))

        def cp_out(c, r0=0, r1=T):
            sl, rs = pl.ds(c * NC, NC), pl.ds(r0, r1 - r0)
            return pltpu.make_async_copy(out_v.at[rs, sl], out_hbm.at[rs, sl],
                                         sems.at[n_sems - 1])

        q_bufs, o_bufs = (q_a, q_b), (o_a, o_b)
        q_cov = {g: {c: set() for c in range(NCQ)} for g in range(Hkv)}
        o_cov = {g: set() for g in range(Hkv)}
        s_issued = {g: set() for g in range(Hkv)}
        c_issued = {g: set() for g in range(Hkv)}

        def q_ready(g, b):
            rows = set(range(b * Sq, (b + 1) * Sq))
            return all(rows <= q_cov[g][c] for c in range(NCQ))

        def B_chunk(g, c, r0=0, r1=T):
            need(("wq", g), ("x", -1), ("x", 0))
            assert g < 2 or len(s_issued[g - 2]) == B, "q buffer overwritten too early"
            q_cov[g][c].update(range(r0, r1))
            sl = slice(c * NC, (c + 1) * NC)
            q = jnp.dot(x_v[r0:r1, :], wq_v[g, :, sl], preferred_element_type=jnp.float32)
            q_bufs[g % 2][r0:r1, sl] = q.astype(jnp.bfloat16)

        def A_S_mm(g, b):
            need(("k", g))
            assert q_ready(g, b), ("q read before written", g, b)
            s_issued[g].add(b)
            q_ref = q_bufs[g % 2]
            Q = jnp.concatenate(
                [q_ref[b * Sq:(b + 1) * Sq, j * Dh:(j + 1) * Dh] for j in range(rep)], axis=0)
            return jax.lax.dot_general(k_v[g, b], Q, (((1,), (1,)), ((), ())),
                                       preferred_element_type=jnp.float32)

        def A_S_softmax(st):
            m = jnp.max(st, axis=0, keepdims=True)
            e = jnp.exp2((st - m) * exp2_scale)
            l = jnp.sum(e, axis=0, keepdims=True)
            return (e * (1.0 / l)).astype(jnp.bfloat16).T

        def A_PV(g, b, p):
            need(("v", g))
            assert g < 2 or len(c_issued[g - 2]) == NCO * T, "o buffer overwritten too early"
            o_cov[g].update(range(b * Sq, (b + 1) * Sq))
            o_ref = o_bufs[g % 2]
            for j in range(rep):
                O = jnp.dot(p[j * Sq:(j + 1) * Sq, :], v_v[g, b],
                            preferred_element_type=jnp.float32)
                o_ref[b * Sq:(b + 1) * Sq, j * Dh:(j + 1) * Dh] = O.astype(jnp.bfloat16)

        def C_chunk(g, c, r0=0, r1=T):
            need(("wo", g))
            assert set(range(r0, r1)) <= o_cov[g], ("o read before written", g)
            c_issued[g].update((c, r) for r in range(r0, r1))
            sl = slice(c * NC, (c + 1) * NC)
            contrib = jnp.dot(o_bufs[g % 2][r0:r1, :], wo_v[g, :, sl],
                              preferred_element_type=jnp.float32)
            if g == 0:
                acc[r0:r1, sl] = contrib
            elif g < Hkv - 1:
                acc[r0:r1, sl] += contrib
            else:
                out_v[r0:r1, sl] = (acc[r0:r1, sl] + contrib).astype(out_v.dtype)

        def fillers(s):
            if s == 1 or s == Hkv:
                fn, g, n = (B_chunk, s, NCQ) if s == 1 else (C_chunk, s - 2, NCO)
                return [functools.partial(fn, g, c, h * (T // 2), (h + 1) * (T // 2))
                        for h in range(2) for c in range(n)]
            fs = []
            if s < Hkv:
                fs += [functools.partial(B_chunk, s, c) for c in range(NCQ)]
            if s >= 2:
                fs += [functools.partial(C_chunk, s - 2, c) for c in range(NCO)]
            return fs

        start(-1)
        start(0)
        start(1)
        wait_group(-1)
        qpart[...] = jnp.dot(x_v[:, 0:KH], wq_v[0, 0:KH, :], preferred_element_type=jnp.float32)
        wait_group(0)
        start(2)
        q_a[...] = (qpart[...] + jnp.dot(x_v[:, KH:], wq_v[0, KH:, :],
                                       preferred_element_type=jnp.float32)).astype(jnp.bfloat16)

        for c in range(NCQ):
            q_cov[0][c].update(range(T))

        p_vals, pending = {}, []

        def issue_S(g, b):
            if (g, b) not in p_vals:
                p_vals[(g, b)] = A_S_softmax(A_S_mm(g, b))

        for s in range(1, Hkv + 2):
            if s in barrier_stages:
                wait_group(s)
            for b, st in pending:
                p_vals[(s - 1, b)] = A_S_softmax(st)
            pending = []
            fs = fillers(s)
            if s <= Hkv:
                a = s - 1
                la, lag = (3, 1) if s == 1 else (2, 0)
                for b in range(la):
                    issue_S(a, b)
                for i in range(B):
                    for b in starts.get((s, i), ()):
                        start(b)
                    nb = i + la
                    if nb < B:
                        issue_S(a, nb)
                    elif (a + 1 < Hkv and (s + 1) not in barrier_stages and nb - B < 2
                          and q_ready(a + 1, nb - B)):
                        issue_S(a + 1, nb - B)
                    lo, hi = i * len(fs) // B, (i + 1) * len(fs) // B
                    for f in fs[lo:hi]:
                        f()
                    if i >= lag:
                        A_PV(a, i - lag, p_vals.pop((a, i - lag)))
                for i in range(B - lag, B):
                    A_PV(a, i, p_vals.pop((a, i)))
                if (s + 1) in barrier_stages and (a + 1) in early_k:
                    pending = [(b, A_S_mm(a + 1, b)) for b in range(min(LB, B))
                               if (a + 1, b) not in p_vals and q_ready(a + 1, b)]
            else:
                for c in range(NCO):
                    if c == NCO - 1 and RT < T:
                        C_chunk(Hkv - 1, c, 0, RT)
                        cp_out(c, 0, RT).start()
                        C_chunk(Hkv - 1, c, RT, T)
                        cp_out(c, RT, T).start()
                    else:
                        C_chunk(Hkv - 1, c)
                        cp_out(c).start()
        for c in range(NCO):
            if c == NCO - 1 and RT < T:
                cp_out(c, 0, RT).wait()
                cp_out(c, RT, T).wait()
            else:
                cp_out(c).wait()
        assert started == set(group_of) and waited == started and not p_vals

    x2 = x.reshape(T, D)
    bf = x.dtype
    out = pl.pallas_call(
        kernel_function,
        in_specs=[pl.BlockSpec(memory_space=pl.ANY)] * 5,
        out_specs=pl.BlockSpec(memory_space=pl.ANY),
        out_shape=jax.ShapeDtypeStruct((T, D), x.dtype),
        scratch_shapes=[
            pltpu.VMEM((T, D), bf),
            pltpu.VMEM((Hkv, B, Sk, Dh), bf),
            pltpu.VMEM((Hkv, B, Sk, Dh), bf),
            pltpu.VMEM((Hkv, D, G), bf),
            pltpu.VMEM((Hkv, G, D), bf),
            pltpu.VMEM((T, G), bf),
            pltpu.VMEM((T, G), bf),
            pltpu.VMEM((T, G), bf),
            pltpu.VMEM((T, G), bf),
            pltpu.VMEM((T, D), jnp.float32),
            pltpu.VMEM((T, D), bf),
            pltpu.VMEM((T, G), jnp.float32),
            pltpu.SemaphoreType.DMA((n_sems,)),
        ],
        compiler_params=pltpu.CompilerParams(
            vmem_limit_bytes=96 * 1024 * 1024,
        ),
    )(x2, k_cache, v_cache, wq, wo)
    return out.reshape(B, Sq, D)
```
